```python
import os as _os
_os.environ.setdefault("JAX_PLATFORMS", "cpu")
import jax
import jax.numpy as jnp

def _softmax(x, axis=-1):
    return jax.nn.softmax(x, axis=axis)
def _gelu(x):
    return jax.nn.gelu(x, approximate=True)
def _silu(x):
    return jax.nn.silu(x)
def _sigmoid(x):
    return jax.nn.sigmoid(x)
def _layernorm(x, axis=-1, eps=1e-5):
    m = jnp.mean(x, axis=axis, keepdims=True)
    v = jnp.var(x, axis=axis, keepdims=True)
    return (x - m) / jnp.sqrt(v + eps)
def _scatter_add(tgt, idx, src, axis=0):
    return tgt.at[idx].add(src)
def _segment_sum(src, seg, n):
    return jax.ops.segment_sum(src, seg, n)
class _Rng:
    def __init__(self, key):
        self._k = key
    def _next(self):
        self._k, sub = jax.random.split(self._k)
        return sub
    def normal(self, shape):
        return jax.random.normal(self._next(), shape, dtype=jnp.bfloat16)
    def randint(self, lo, hi, shape):
        return jax.random.randint(self._next(), shape, lo, hi, dtype=jnp.int32)
    def uniform(self, shape, lo=0.0, hi=1.0):
        return jax.random.uniform(self._next(), shape, jnp.bfloat16, lo, hi)
    def permutation(self, n):
        return jax.random.permutation(self._next(), n)


kernel_name = 'standalone__seq2seq_rnn_t_joint__speech'

def setup_inputs():
    _rng = _Rng(jax.random.key(int.from_bytes(__import__("os").urandom(4), "little")))
    _w = (lambda a: (lambda t: t.astype(jnp.bfloat16) if jnp.issubdtype(t.dtype, jnp.floating) else t)(jnp.asarray(a)))
    B, T, D, K = 2, 16000, 256, 31
    U = 8
    sc = (1.0 / (K * D)) ** 0.5
    sd = (1.0 / D) ** 0.5
    return {
        "x": _w((lambda *s: _rng.normal(s) * 0.2)(B, T, D) * 0.5),
        "w1": _w((lambda *s: _rng.normal(s) * 1.6)(K, D, D) * sc),
        "w2": _w((lambda *s: _rng.normal(s) * 1.6)(K, D, D) * sc),
        "g": _w((lambda *s: _rng.normal(s) * 1.6)(B, U, D) * 0.5),
        "w_f": _w((lambda *s: _rng.normal(s) * 1.6)(D, D) * sd),
        "w_g": _w((lambda *s: _rng.normal(s) * 1.6)(D, D) * sd),
        "w_o": _w((lambda *s: _rng.normal(s) * 1.6)(D, D) * sd),
    }

def reference(x, w1, w2, g, w_f, w_g, w_o):
    B, T, D = x.shape
    K = w1.shape[0]
    pad = K // 2
    xp = jnp.pad(x, ((0,0),(pad,pad),(0,0)))
    h = jnp.zeros_like(x)
    for i in range(K):
        h = h + jnp.einsum("btc,cd->btd", xp[:, i:i+T, :], w1[i])
    h = _gelu(h)[:, ::2, :]
    T1 = h.shape[1]
    hp = jnp.pad(h, ((0,0),(pad,pad),(0,0)))
    f = jnp.zeros_like(h)
    for i in range(K):
        f = f + jnp.einsum("btc,cd->btd", hp[:, i:i+T1, :], w2[i])
    f = _gelu(f)[:, ::2, :]
    fe = jnp.einsum("btd,de->bte", f, w_f)
    ge = jnp.einsum("bud,de->bue", g, w_g)
    j = jnp.tanh(fe[:, :, None, :] + ge[:, None, :, :])
    return jnp.einsum("btud,dv->btuv", j, w_o)
```

```python
import functools

import jax
import jax.numpy as jnp
from jax import lax
import jax.experimental.pallas as pl
import jax.experimental.pallas.tpu as pltpu

F32 = jnp.float32
BF16 = jnp.bfloat16
U32 = jnp.uint32

B, T, D, KT, NU = 2, 16000, 256, 31, 8
NB1 = 336
NB2 = 168
XB = 48
XSTRIDE = NB1 * 48
FSTRIDE = NB2 * 24
T1 = T // 2
T2 = T // 4
HPAD = 8

BR_ORDER = (1, 2, 0, 3)
INNER = [(a2, a3, a4) for a2 in (1, 0, 2) for a3 in (1, 0, 2) for a4 in (1, 0, 2)]


def _is_raw(a1, a):
    return a1 in (0, 3) and all(v != 1 for v in a)


_USLOT = {}
for _a1 in range(4):
    for _a in INNER:
        if not _is_raw(_a1, _a):
            _USLOT[(_a1,) + _a] = len(_USLOT)
NUSLOT = len(_USLOT)


def _sgn(t):
    return (-1) ** sum(1 for v in t if v == 2)


def _prod_of(sset, off):
    base = sum(d for d in (4, 2, 1) if d not in sset)
    rem = off - base
    return tuple((2 if rem & d else 0) if d in sset else 1 for d in (4, 2, 1))


def _gelu_signed(v, sgn):
    c0 = 0.7978845608028654 * sgn
    c1 = 0.7978845608028654 * 0.044715 * sgn
    inner = v * (c0 + c1 * (v * v))
    hx = (0.5 * sgn) * v
    return hx + hx * jnp.tanh(inner)


class Cfg:
    def __init__(self, MC1=48, MC2=48, JB=800, JS=200, xwait=(0, 1, 3, 7), NWP=4,
                 scopes=False, x0at=2):
        self.MC1, self.MC2 = MC1, MC2
        self.NS1 = B * NB1 // MC1
        self.NS2 = B * NB2 // MC2
        self.XSR = 2 * MC1 + 8
        self.JB, self.JS = JB, JS
        self.scopes = scopes
        self.NWP = NWP
        self.x0at = x0at
        self.X_ROWS = 2 * (8 + 24 * MC1 * (self.NS1 - 1) + 12 * self.XSR + 8)
        self.H_ROWS = HPAD + B * NB1 + 8
        self.xwait = tuple(k for k in xwait if k < self.NS1)
        pieces, done = [], 0
        for i, k in enumerate(self.xwait):
            kl = (self.xwait[i + 1] if i + 1 < len(self.xwait) else self.NS1) - 1
            need = 24 * (2 * MC1 * kl - 1 + self.XSR)
            need = -(-need // 16) * 16
            if kl == self.NS1 - 1:
                need = B * XSTRIDE
            cur = []
            for b in range(B):
                lo = max(done - b * XSTRIDE, 0)
                hi = min(need - b * XSTRIDE, T)
                if hi > lo:
                    cur.append((b, lo, hi))
            done = need
            pieces.append(cur)
        self.X_PIECES = pieces
        self.N_XSEM = 2 * sum(len(p) for p in pieces)


class _NoScope:
    def __enter__(self):
        return self

    def __exit__(self, *a):
        return False


def _kernel(x_hbm, w1_hbm, w2_hbm, g_hbm, wf_hbm, wg_hbm, wo_hbm, o_hbm,
            raw_ref, xs_ref, hs_ref, f_ref, u_ref, ob_ref, wr1_ref, wr2_ref,
            g_ref, wf_ref, wg_ref, wo_ref, ge_ref,
            xsem, wsem, ssem, osem, *, cfg):
    MC1, MC2, NS1, NS2, XSR, NWP = cfg.MC1, cfg.MC2, cfg.NS1, cfg.NS2, cfg.XSR, cfg.NWP
    scope = (lambda n: jax.named_scope(n)) if cfg.scopes else (lambda n: _NoScope())
    raw_u = raw_ref.bitcast(U32)
    f_u = f_ref.bitcast(U32)
    u_u = u_ref.bitcast(U32)

    def x_copies(k):
        out = []
        si = 2 * sum(len(p) for p in cfg.X_PIECES[:k])
        for (b, lo, hi) in cfg.X_PIECES[k]:
            for h in range(2):
                out.append(pltpu.make_async_copy(
                    x_hbm.at[b, pl.ds(lo, hi - lo), pl.ds(128 * h, 128)],
                    raw_ref.at[h, pl.ds(XB + b * XSTRIDE + lo, hi - lo), :],
                    xsem.at[si]))
                si += 1
        return out

    WR = D // NWP

    def w1_copies(i):
        r0 = i * WR
        if not isinstance(r0, int):
            r0 = pl.multiple_of(r0, WR)
        return [pltpu.make_async_copy(
            w1_hbm.at[:, pl.ds(r0, WR), pl.ds(128 * h, 128)],
            wr1_ref.at[h, :, pl.ds(r0, WR), :], wsem.at[2 * i + h]) for h in range(2)]

    w2_copies = [pltpu.make_async_copy(
        w2_hbm.at[:, :, pl.ds(128 * h, 128)], wr2_ref.at[h], wsem.at[2 * NWP + h])
        for h in range(2)]

    small = [pltpu.make_async_copy(s, d, ssem.at[i]) for i, (s, d) in enumerate(
        [(g_hbm, g_ref), (wf_hbm, wf_ref), (wg_hbm, wg_ref), (wo_hbm, wo_ref)])]

    for i in range(2):
        for c in w1_copies(i):
            c.start()

    def zero_raw(lo, hi):
        for h in range(2):
            raw_u[h, pl.ds(lo // 2, (hi - lo) // 2), :] = jnp.zeros(((hi - lo) // 2, 128), U32)

    zero_raw(0, XB)
    zero_raw(XB + T, XB + XSTRIDE)
    zero_raw(XB + XSTRIDE + T, cfg.X_ROWS)
    hs_ref[:, :, pl.ds(0, HPAD), :] = jnp.zeros((12, 2, HPAD, 128), U32)
    hs_ref[:, :, pl.ds(HPAD + B * NB1, 8), :] = jnp.zeros((12, 2, 8, 128), U32)

    def w_unit(wr_u, rg, ph, h, branches):
        r0 = pl.multiple_of(rg * 8, 8)
        u0 = pl.multiple_of(ph * 256 + rg * 16, 16)

        def tap(j):
            if 2 * j - 1 + ph < 0:
                return jnp.zeros((16, 128), F32)
            tu = wr_u[h, 2 * j - 1 + ph, pl.ds(r0, 8), :]
            return pltpu.bitcast(tu, BF16).astype(F32)

        def rec(a1, level_d, ws, prefix):
            if level_d == 0:
                if not _is_raw(a1, prefix):
                    u_ref[_USLOT[(a1,) + prefix], h, pl.ds(u0, 16), :] = ws[0].astype(BF16)
                return
            lo, hi = ws[:level_d], ws[level_d:]
            rec(a1, level_d // 2, lo, prefix + (0,))
            rec(a1, level_d // 2, [a + b for a, b in zip(lo, hi)], prefix + (1,))
            rec(a1, level_d // 2, hi, prefix + (2,))

        lo = [tap(j) for j in range(8)]
        hi = [tap(j + 8) for j in range(8)]
        for a1 in branches:
            if a1 == 0:
                rec(0, 4, lo, ())
            elif a1 == 3:
                rec(3, 4, hi, ())
            elif a1 == 1:
                rec(1, 4, [(a + b) * 0.5 for a, b in zip(lo, hi)], ())
            else:
                rec(2, 4, [(a - b) * 0.5 for a, b in zip(lo, hi)], ())

    def w_rows(wr_u, rg_lo, rg_hi):
        for branches in ((1, 2), (0, 3)):
            def body(rg, carry, branches=branches):
                for ph in range(2):
                    for h in range(2):
                        w_unit(wr_u, rg, ph, h, branches)
                return carry
            lax.fori_loop(rg_lo, rg_hi, body, 0)

    def t_unit(st_ref, roff, branch, g, l, vals):
        ph, h = l // 2, l % 2

        def X(i):
            dl, r = divmod(2 * i + ph - 16, 24)
            u = st_ref[r // 2, h, pl.ds(32 * g + dl + roff, 16, stride=2), :]
            u = (u & jnp.uint32(0xFFFF0000)) if ph else (u << 16)
            return lax.bitcast_convert_type(u, F32)

        def Z(i):
            if branch == 0:
                return X(i) - X(i + 16)
            if branch == 1:
                return X(i + 8) + X(i + 16)
            if branch == 2:
                return X(i + 16) - X(i + 8)
            return X(i + 8) - X(i + 24)

        def put(sset, off, val):
            vals[(_prod_of(sset, off), g, l)] = val

        z, a, b, d2 = {}, {}, {}, {}
        for n in range(15):
            z[n] = Z(n)
            if n == 7:
                put((), 7, z[7])
            if n - 1 in (6, 7):
                put((1,), n - 1, z[n - 1] - z[n])
            if 4 <= n - 2 <= 8:
                d2[n - 2] = z[n - 2] - z[n]
                if n - 2 in (5, 7):
                    put((2,), n - 2, d2[n - 2])
            if 4 <= n - 3 <= 7:
                put((2, 1), n - 3, d2[n - 3] - d2[n - 2])
            if n >= 4:
                a[n - 4] = z[n - 4] - z[n]
                if n - 4 in (3, 7):
                    put((4,), n - 4, a[n - 4])
            if n - 5 in (2, 3, 6, 7):
                put((4, 1), n - 5, a[n - 5] - a[n - 4])
            if n >= 6:
                b[n - 6] = a[n - 6] - a[n - 4]
                if n - 6 in (1, 3, 5, 7):
                    put((4, 2), n - 6, b[n - 6])
            if n >= 7:
                put((4, 2, 1), n - 7, b[n - 7] - b[n - 6])

    def mm_branch(mc, wr_u, branch, vals, qv, store_out):
        pv = {}
        for a in INNER:
            a2, a3, a4 = a
            s_in = _sgn(a)
            l0 = 0
            if _is_raw(branch, a):
                j = 8 * (branch // 3) + 4 * (a2 // 2) + 2 * (a3 // 2) + a4 // 2
                taps = [2 * j - 1, 2 * j]
                if j == 0:
                    taps, l0 = [0], 2
                rhs_u = jnp.concatenate(
                    [jnp.concatenate([wr_u[h, t] for t in taps], axis=0) for h in range(2)],
                    axis=1)
            else:
                rhs_u = jnp.concatenate(
                    [u_u[_USLOT[(branch,) + a], h] for h in range(2)], axis=1)
            lhs = jnp.concatenate(
                [jnp.concatenate([vals[(a, g, l)] for l in range(l0, 4)], axis=1)
                 for g in range(mc // 16)], axis=0).astype(BF16)
            val = jnp.dot(lhs, pltpu.bitcast(rhs_u, BF16), preferred_element_type=F32)
            deps = []
            if a4 != 1:
                deps.append((a2, a3, 1))
                if a3 != 1:
                    deps.append((a2, 1, a4))
                    if a2 != 1:
                        deps.append((1, a3, a4))
            for dslot in deps:
                if _sgn(dslot) == s_in:
                    val = val + pv[dslot]
                else:
                    val = val - pv[dslot]
            if len(deps) < 3:
                pv[a] = val
                continue
            rp = (a2 // 2) * 4 + (a3 // 2) * 2 + (a4 // 2)
            if branch == 1:
                qv[rp] = val
                continue
            if branch == 2:
                y, o = qv[rp] - val, 1
                qv[rp] = qv[rp] + val
            elif branch == 0:
                y, o = qv[rp] + val, 0
            else:
                y, o = qv[rp] - val, 2
            gl = _gelu_signed(y, float(s_in))
            if a4 == 0:
                pv[a] = gl
                continue
            ev = pv[(a2, a3, 0)]
            lo = lax.bitcast_convert_type(ev.astype(BF16).astype(F32), U32) >> 16
            hi = lax.bitcast_convert_type(gl.astype(BF16).astype(F32), U32)
            pk = hi | lo
            for h in range(2):
                store_out(4 * o + rp // 2, h, pk[:, 128 * h:128 * (h + 1)])

    def conv_block(mc, wr_u, st_ref, roff, store_out):
        qv = {}
        for br in BR_ORDER:
            vals = {}
            for g in range(mc // 16):
                for l in range(4):
                    t_unit(st_ref, roff, br, g, l, vals)
            mm_branch(mc, wr_u, br, vals, qv, store_out)

    wr1_u = wr1_ref.bitcast(U32)
    wr2_u = wr2_ref.bitcast(U32)
    per = 16 // NWP

    def w1_piece(i, carry):
        for c in w1_copies(i):
            c.wait()

        @pl.when(i + 2 < NWP)
        def _():
            for c in w1_copies(i + 2):
                c.start()

        @pl.when(i == cfg.x0at)
        def _():
            for c in x_copies(0):
                c.start()
        w_rows(wr1_u, i * per, (i + 1) * per)
        return carry

    with scope("ph_w1"):
        lax.fori_loop(0, NWP, w1_piece, 0)

    def conv1_body(s, carry):
        for k, sk in enumerate(cfg.xwait):
            @pl.when(s == sk)
            def _():
                with scope("ph_xwait"):
                    for c in x_copies(k):
                        c.wait()
                if k + 1 < len(cfg.X_PIECES):
                    for c in x_copies(k + 1):
                        c.start()
                if k == len(cfg.X_PIECES) - 1:
                    for c in w2_copies + small:
                        c.start()

        srcb = pl.multiple_of(8 + (24 * MC1) * s, 8)
        src = raw_u.at[:, pl.ds(srcb, 12 * XSR + 8), :]
        for g in range(MC1 // 16):
            r0, n = (0, 40) if g == 0 else (32 * g + 8, 32)
            for q in range(12):
                for h in range(2):
                    xs_ref[q, h, pl.ds(r0, n), :] = src[
                        h, pl.ds(4 + q + 12 * r0, n, stride=12), :]

        hb = pl.multiple_of(HPAD + MC1 * s, 8)

        def store_h(qq, h, val):
            hs_ref[qq, h, pl.ds(hb, MC1), :] = val

        conv_block(MC1, wr1_u, xs_ref, 1, store_h)
        return carry

    with scope("ph_conv1"):
        lax.fori_loop(0, NS1, conv1_body, 0)

    for c in w2_copies:
        c.wait()
    with scope("ph_w2"):
        w_rows(wr2_u, 0, 16)

    nfull, rem = divmod(T1, 24)
    for b in range(B):
        r0 = HPAD + b * NB1 + nfull
        hs_ref[pl.ds(rem // 2, 12 - rem // 2), :, pl.ds(r0, 1), :] = jnp.zeros(
            (12 - rem // 2, 2, 1, 128), U32)
        hs_ref[:, :, pl.ds(r0 + 1, NB1 - nfull - 1), :] = jnp.zeros(
            (12, 2, NB1 - nfull - 1, 128), U32)

    JB, JS = cfg.JB, cfg.JS
    NSUB = JB // JS
    NJB = T2 // JB
    for c in small:
        c.wait()
    for b in range(B):
        ge_ref[b] = jnp.dot(g_ref[b], wg_ref[...], preferred_element_type=F32)

    def out_copy(slot, sub, b, t0):
        return pltpu.make_async_copy(
            ob_ref.at[slot, pl.ds(sub * JS, JS)], o_hbm.at[b, pl.ds(t0 + sub * JS, JS)],
            osem.at[slot * NSUB + sub])

    def jbody(gi, carry):
        b = gi // NJB
        t0 = (gi % NJB) * JB
        slot = gi % 2

        @pl.when(gi >= 2)
        def _():
            for sub in range(NSUB):
                out_copy(slot, sub, b, t0).wait()

        ge = ge_ref[b]
        r0 = pl.multiple_of((b * FSTRIDE + t0) // 2, 8)
        fsrc = f_u.at[:, pl.ds(r0, JB // 2), :]
        f = jnp.concatenate(
            [pltpu.bitcast(fsrc[h], BF16) for h in range(2)], axis=1)
        fe = jnp.dot(f, wf_ref[...], preferred_element_type=F32)
        for sub in range(NSUB):
            fs = fe[sub * JS:(sub + 1) * JS]
            jj = jnp.tanh(fs[:, None, :] + ge[None, :, :]).reshape(JS * NU, D).astype(BF16)
            o = jnp.dot(jj, wo_ref[...], preferred_element_type=F32)
            ob_ref[slot, pl.ds(sub * JS, JS)] = o.reshape(JS, NU, D).astype(BF16)
            out_copy(slot, sub, b, t0).start()
        return carry

    def conv2_body(c, done):
        hb = pl.multiple_of(2 * MC2 * c, 8)
        hsv = hs_ref.at[:, :, pl.ds(hb, 2 * MC2 + 16), :]
        fb = pl.multiple_of(12 * MC2 * c, 8)
        dst = f_u.at[:, pl.ds(fb, 12 * MC2), :]

        def store_f(qq, h, val):
            dst[h, pl.ds(qq, MC2, stride=12), :] = val

        with scope("ph_conv2"):
            conv_block(MC2, wr2_u, hsv, HPAD, store_f)
        avail = 24 * MC2 * (c + 1)
        ready = 0
        for b in range(B):
            ready = ready + jnp.clip(jnp.maximum(avail - b * FSTRIDE, 0) // JB, 0, NJB)
        with scope("ph_joint"):
            lax.fori_loop(done, ready, jbody, 0)
        return ready

    lax.fori_loop(0, NS2, conv2_body, 0)
    with scope("ph_tail"):
        for slot in range(2):
            for sub in range(NSUB):
                out_copy(slot, sub, 0, 0).wait()


_CFG = Cfg()


@jax.jit
def pallas_standalone__seq2seq_rnn_t_joint__speech_kernel(x, w1, w2, g, w_f, w_g, w_o):
    cfg = _CFG
    anyspec = pl.BlockSpec(memory_space=pl.ANY)
    return pl.pallas_call(
        functools.partial(_kernel, cfg=cfg),
        out_shape=jax.ShapeDtypeStruct((B, T2, NU, D), BF16),
        in_specs=[anyspec] * 7,
        out_specs=anyspec,
        scratch_shapes=[
            pltpu.VMEM((2, cfg.X_ROWS, 128), BF16),
            pltpu.VMEM((12, 2, cfg.XSR, 128), U32),
            pltpu.VMEM((12, 2, cfg.H_ROWS, 128), U32),
            pltpu.VMEM((2, B * FSTRIDE, 128), BF16),
            pltpu.VMEM((NUSLOT, 2, 512, 128), BF16),
            pltpu.VMEM((2, cfg.JB, NU, D), BF16),
            pltpu.VMEM((2, KT, D, 128), BF16),
            pltpu.VMEM((2, KT, D, 128), BF16),
            pltpu.VMEM((B, NU, D), BF16),
            pltpu.VMEM((D, D), BF16),
            pltpu.VMEM((D, D), BF16),
            pltpu.VMEM((D, D), BF16),
            pltpu.VMEM((B, NU, D), F32),
            pltpu.SemaphoreType.DMA((cfg.N_XSEM,)),
            pltpu.SemaphoreType.DMA((2 * cfg.NWP + 2,)),
            pltpu.SemaphoreType.DMA((4,)),
            pltpu.SemaphoreType.DMA((2 * (cfg.JB // cfg.JS),)),
        ],
        compiler_params=pltpu.CompilerParams(vmem_limit_bytes=110 * 1024 * 1024),
    )(x, w1, w2, g, w_f, w_g, w_o)
```

```python
import functools

import jax
import jax.numpy as jnp
from jax import lax
import jax.experimental.pallas as pl
import jax.experimental.pallas.tpu as pltpu

F32 = jnp.float32
BF16 = jnp.bfloat16
U32 = jnp.uint32

B, T, D, KT, NU = 2, 16000, 256, 31, 8
T1 = T // 2
T2 = T // 4
NB1 = 336
NB2 = 168
MC = 48
NS1 = B * NB1 // MC
NS2 = B * NB2 // MC
XB = 48
XSTRIDE = NB1 * 48
FSTRIDE = NB2 * 24
XSR = 2 * MC + 8
SRCV = 12 * XSR + 32
X_ROWS = -(-2 * (24 * MC * (NS1 - 1) + SRCV) // 64) * 64
HPAD = 8
H_ROWS = HPAD + B * NB1 + 8
UROWS = 512 + 16
NWP = 4
XWAIT = (0, 1, 3, 7)
JB = 800
JS = 200
NSUB = JB // JS
NJB = T2 // JB

BR_ORDER = (1, 2, 0, 3)
INNER = [(a2, a3, a4) for a2 in (1, 0, 2) for a3 in (1, 0, 2) for a4 in (1, 0, 2)]


def _is_raw(a1, a):
    return a1 in (0, 3) and all(v != 1 for v in a)


_USLOT = {}
for _a1 in range(4):
    for _a in INNER:
        if not _is_raw(_a1, _a):
            _USLOT[(_a1,) + _a] = len(_USLOT)
NUSLOT = len(_USLOT)


def _x_pieces():
    pieces, done = [], 0
    for i in range(len(XWAIT)):
        last = (XWAIT[i + 1] if i + 1 < len(XWAIT) else NS1) - 1
        need = 2 * (24 * MC * last + SRCV) - XB
        if last == NS1 - 1:
            need = B * XSTRIDE
        cur = []
        for b in range(B):
            lo = max(done - b * XSTRIDE, 0)
            hi = min(need - b * XSTRIDE, T)
            if hi > lo:
                cur.append((b, lo, hi))
        done = need
        pieces.append(cur)
    return pieces


X_PIECES = _x_pieces()
N_XSEM = 2 * sum(len(p) for p in X_PIECES)


def _sgn(t):
    return (-1) ** sum(1 for v in t if v == 2)


def _prod_of(sset, off):
    base = sum(d for d in (4, 2, 1) if d not in sset)
    rem = off - base
    return tuple((2 if rem & d else 0) if d in sset else 1 for d in (4, 2, 1))


def _gelu_scaled(v, k):
    c0 = 0.7978845608028654 * k
    c1 = 0.7978845608028654 * 0.044715 * k * k * k
    inner = v * (c0 + c1 * (v * v))
    hx = (0.5 * k) * v
    return hx + hx * jnp.tanh(inner)


def _kernel(x_hbm, w1_hbm, w2_hbm, g_hbm, wf_hbm, wg_hbm, wo_hbm, o_hbm,
            raw_ref, xs_ref, hs_ref, f_ref, u_ref, ob_ref, wr1_ref, wr2_ref,
            g_ref, wf_ref, wg_ref, wo_ref, ge_ref,
            xsem, wsem, ssem, osem):
    raw_u = raw_ref.bitcast(U32)
    f_u = f_ref.bitcast(U32)
    u_u = u_ref.bitcast(U32)
    wr1_u = wr1_ref.bitcast(U32)
    wr2_u = wr2_ref.bitcast(U32)

    def x_copies(k):
        out = []
        si = 2 * sum(len(p) for p in X_PIECES[:k])
        for (b, lo, hi) in X_PIECES[k]:
            for h in range(2):
                out.append(pltpu.make_async_copy(
                    x_hbm.at[b, pl.ds(lo, hi - lo), pl.ds(128 * h, 128)],
                    raw_ref.at[h, pl.ds(XB + b * XSTRIDE + lo, hi - lo), :],
                    xsem.at[si]))
                si += 1
        return out

    wrows = D // NWP

    def w1_copies(i):
        r0 = i * wrows
        if not isinstance(r0, int):
            r0 = pl.multiple_of(r0, wrows)
        return [pltpu.make_async_copy(
            w1_hbm.at[:, pl.ds(r0, wrows), pl.ds(128 * h, 128)],
            wr1_ref.at[h, :, pl.ds(r0, wrows), :], wsem.at[2 * i + h]) for h in range(2)]

    w2_copies = [pltpu.make_async_copy(
        w2_hbm.at[:, :, pl.ds(128 * h, 128)], wr2_ref.at[h], wsem.at[2 * NWP + h])
        for h in range(2)]

    small = [pltpu.make_async_copy(s, d, ssem.at[i]) for i, (s, d) in enumerate(
        [(g_hbm, g_ref), (wf_hbm, wf_ref), (wg_hbm, wg_ref), (wo_hbm, wo_ref)])]

    for i in range(2):
        for c in w1_copies(i):
            c.start()

    def zero_raw(lo, hi):
        for h in range(2):
            raw_u[h, pl.ds(lo // 2, (hi - lo) // 2), :] = jnp.zeros(((hi - lo) // 2, 128), U32)

    zero_raw(0, XB)
    zero_raw(XB + T, XB + XSTRIDE)
    zero_raw(XB + XSTRIDE + T, X_ROWS)
    hs_ref[:, :, pl.ds(0, HPAD), :] = jnp.zeros((12, 2, HPAD, 128), U32)
    hs_ref[:, :, pl.ds(HPAD + B * NB1, 8), :] = jnp.zeros((12, 2, 8, 128), U32)

    def w_unit(wr_u, rg, ph, h, branches):
        r0 = pl.multiple_of(rg * 8, 8)
        u0 = pl.multiple_of(ph * 256 + rg * 16, 16)

        def tap(j):
            if 2 * j - 1 + ph < 0:
                return jnp.zeros((16, 128), F32)
            tu = wr_u[h, 2 * j - 1 + ph, pl.ds(r0, 8), :]
            return pltpu.bitcast(tu, BF16).astype(F32)

        def rec(a1, d, ws, prefix):
            if d == 0:
                if not _is_raw(a1, prefix):
                    u_ref[_USLOT[(a1,) + prefix], h, pl.ds(u0, 16), :] = ws[0].astype(BF16)
                return
            lo, hi = ws[:d], ws[d:]
            rec(a1, d // 2, lo, prefix + (0,))
            rec(a1, d // 2, [a + b for a, b in zip(lo, hi)], prefix + (1,))
            rec(a1, d // 2, hi, prefix + (2,))

        lo = [tap(j) for j in range(8)]
        hi = [tap(j + 8) for j in range(8)]
        for a1 in branches:
            if a1 == 0:
                rec(0, 4, lo, ())
            elif a1 == 3:
                rec(3, 4, hi, ())
            elif a1 == 1:
                rec(1, 4, [a + b for a, b in zip(lo, hi)], ())
            else:
                rec(2, 4, [a - b for a, b in zip(lo, hi)], ())

    def w_rows(wr_u, rg_lo, rg_hi):
        for branches in ((1, 2), (0, 3)):
            def body(rg, carry, branches=branches):
                for ph in range(2):
                    for h in range(2):
                        w_unit(wr_u, rg, ph, h, branches)
                return carry
            lax.fori_loop(rg_lo, rg_hi, body, 0)

    def t_unit(st_ref, roff, branch, g, l, vals):
        ph, h = l // 2, l % 2

        def X(i):
            dl, r = divmod(2 * i + ph - 16, 24)
            u = st_ref[r // 2, h, pl.ds(32 * g + dl + roff, 16, stride=2), :]
            u = (u & jnp.uint32(0xFFFF0000)) if ph else (u << 16)
            return lax.bitcast_convert_type(u, F32)

        def Z(i):
            if branch == 0:
                return X(i) - X(i + 16)
            if branch == 1:
                return X(i + 8) + X(i + 16)
            if branch == 2:
                return X(i + 16) - X(i + 8)
            return X(i + 8) - X(i + 24)

        def put(sset, off, val):
            vals[(_prod_of(sset, off), g, l)] = val

        z, a, b, d2 = {}, {}, {}, {}
        for n in range(15):
            z[n] = Z(n)
            if n == 7:
                put((), 7, z[7])
            if n - 1 in (6, 7):
                put((1,), n - 1, z[n - 1] - z[n])
            if 4 <= n - 2 <= 8:
                d2[n - 2] = z[n - 2] - z[n]
                if n - 2 in (5, 7):
                    put((2,), n - 2, d2[n - 2])
            if 4 <= n - 3 <= 7:
                put((2, 1), n - 3, d2[n - 3] - d2[n - 2])
            if n >= 4:
                a[n - 4] = z[n - 4] - z[n]
                if n - 4 in (3, 7):
                    put((4,), n - 4, a[n - 4])
            if n - 5 in (2, 3, 6, 7):
                put((4, 1), n - 5, a[n - 5] - a[n - 4])
            if n >= 6:
                b[n - 6] = a[n - 6] - a[n - 4]
                if n - 6 in (1, 3, 5, 7):
                    put((4, 2), n - 6, b[n - 6])
            if n >= 7:
                put((4, 2, 1), n - 7, b[n - 7] - b[n - 6])

    def mm_branch(wr_u, branch, vals, qv, store_out):
        pv = {}
        for a in INNER:
            a2, a3, a4 = a
            s_in = _sgn(a)
            l0 = 0
            if _is_raw(branch, a):
                j = 8 * (branch // 3) + 4 * (a2 // 2) + 2 * (a3 // 2) + a4 // 2
                taps = [2 * j - 1, 2 * j]
                if j == 0:
                    taps, l0 = [0], 2
                rhs_u = jnp.concatenate(
                    [jnp.concatenate([wr_u[h, t] for t in taps], axis=0) for h in range(2)],
                    axis=1)
            else:
                rhs_u = jnp.concatenate(
                    [u_u[_USLOT[(branch,) + a], h, pl.ds(0, 256), :] for h in range(2)],
                    axis=1)
            lhs = jnp.concatenate(
                [jnp.concatenate([vals[(a, g, l)] for l in range(l0, 4)], axis=1)
                 for g in range(MC // 16)], axis=0).astype(BF16)
            val = jnp.dot(lhs, pltpu.bitcast(rhs_u, BF16), preferred_element_type=F32)
            deps = []
            if a4 != 1:
                deps.append((a2, a3, 1))
                if a3 != 1:
                    deps.append((a2, 1, a4))
                    if a2 != 1:
                        deps.append((1, a3, a4))
            for dslot in deps:
                if _sgn(dslot) == s_in:
                    val = val + pv[dslot]
                else:
                    val = val - pv[dslot]
            if len(deps) < 3:
                pv[a] = val
                continue
            rp = (a2 // 2) * 4 + (a3 // 2) * 2 + (a4 // 2)
            if branch == 1:
                qv[rp] = val
                continue
            scl = 1.0
            if branch == 2:
                y, o, scl = qv[rp] - val, 1, 0.5
                qv[rp] = (qv[rp] + val) * 0.5
            elif branch == 0:
                y, o = qv[rp] + val, 0
            else:
                y, o = qv[rp] - val, 2
            gl = _gelu_scaled(y, scl * s_in)
            if a4 == 0:
                pv[a] = gl
                continue
            ev = pv[(a2, a3, 0)]
            lo = lax.bitcast_convert_type(ev.astype(BF16).astype(F32), U32) >> 16
            hi = lax.bitcast_convert_type(gl.astype(BF16).astype(F32), U32)
            pk = hi | lo
            for h in range(2):
                store_out(4 * o + rp // 2, h, pk[:, 128 * h:128 * (h + 1)])

    def conv_block(wr_u, st_ref, roff, store_out):
        qv = {}
        for br in BR_ORDER:
            vals = {}
            for g in range(MC // 16):
                for l in range(4):
                    t_unit(st_ref, roff, br, g, l, vals)
            mm_branch(wr_u, br, vals, qv, store_out)

    per = 16 // NWP

    def w1_piece(i, carry):
        for c in w1_copies(i):
            c.wait()

        @pl.when(i + 2 < NWP)
        def _():
            for c in w1_copies(i + 2):
                c.start()

        @pl.when(i == NWP - 2)
        def _():
            for c in x_copies(0):
                c.start()
        w_rows(wr1_u, i * per, (i + 1) * per)
        return carry

    lax.fori_loop(0, NWP, w1_piece, 0)

    def conv1_body(s, carry):
        for k, sk in enumerate(XWAIT):
            @pl.when(s == sk)
            def _():
                for c in x_copies(k):
                    c.wait()
                if k + 1 < len(X_PIECES):
                    for c in x_copies(k + 1):
                        c.start()
                else:
                    for c in w2_copies + small:
                        c.start()

        srcb = pl.multiple_of((24 * MC) * s, 32)
        src = raw_u.at[:, pl.ds(srcb, SRCV), :]
        for g in range(MC // 16):
            r0, n = (0, 40) if g == 0 else (32 * g + 8, 32)
            for q in range(12):
                for h in range(2):
                    xs_ref[q, h, pl.ds(r0, n), :] = src[
                        h, pl.ds(12 + q + 12 * r0, n, stride=12), :]

        hb = pl.multiple_of(HPAD + MC * s, 8)

        def store_h(qq, h, val):
            hs_ref[qq, h, pl.ds(hb, MC), :] = val

        conv_block(wr1_u, xs_ref, 1, store_h)
        return carry

    lax.fori_loop(0, NS1, conv1_body, 0)

    for c in w2_copies:
        c.wait()
    w_rows(wr2_u, 0, 16)

    nfull, rem = divmod(T1, 24)
    for b in range(B):
        r0 = HPAD + b * NB1 + nfull
        hs_ref[pl.ds(rem // 2, 12 - rem // 2), :, pl.ds(r0, 1), :] = jnp.zeros(
            (12 - rem // 2, 2, 1, 128), U32)
        hs_ref[:, :, pl.ds(r0 + 1, NB1 - nfull - 1), :] = jnp.zeros(
            (12, 2, NB1 - nfull - 1, 128), U32)

    for c in small:
        c.wait()
    for b in range(B):
        ge_ref[b] = jnp.dot(g_ref[b], wg_ref[...], preferred_element_type=F32)

    def out_copy(slot, sub, b, t0):
        return pltpu.make_async_copy(
            ob_ref.at[slot, pl.ds(sub * JS, JS)], o_hbm.at[b, pl.ds(t0 + sub * JS, JS)],
            osem.at[slot * NSUB + sub])

    def jbody(gi, carry):
        b = gi // NJB
        t0 = (gi % NJB) * JB
        slot = gi % 2

        @pl.when(gi >= 2)
        def _():
            for sub in range(NSUB):
                out_copy(slot, sub, b, t0).wait()

        ge = ge_ref[b]
        r0 = pl.multiple_of((b * FSTRIDE + t0) // 2, 8)
        fsrc = f_u.at[:, pl.ds(r0, JB // 2), :]
        f = jnp.concatenate(
            [pltpu.bitcast(fsrc[h], BF16) for h in range(2)], axis=1)
        fe = jnp.dot(f, wf_ref[...], preferred_element_type=F32)
        for sub in range(NSUB):
            fs = fe[sub * JS:(sub + 1) * JS]
            jj = jnp.tanh(fs[:, None, :] + ge[None, :, :]).reshape(JS * NU, D).astype(BF16)
            o = jnp.dot(jj, wo_ref[...], preferred_element_type=F32)
            ob_ref[slot, pl.ds(sub * JS, JS)] = o.reshape(JS, NU, D).astype(BF16)
            out_copy(slot, sub, b, t0).start()
        return carry

    def conv2_body(c, done):
        hb = pl.multiple_of(2 * MC * c, 32)
        hsv = hs_ref.at[:, :, pl.ds(hb, 2 * MC + 16), :]
        fb = pl.multiple_of(12 * MC * c, 32)
        dst = f_u.at[:, pl.ds(fb, 12 * MC + 16), :]

        def store_f(qq, h, val):
            dst[h, pl.ds(qq, MC, stride=12), :] = val

        conv_block(wr2_u, hsv, HPAD, store_f)
        avail = 24 * MC * (c + 1)
        ready = 0
        for b in range(B):
            ready = ready + jnp.clip(jnp.maximum(avail - b * FSTRIDE, 0) // JB, 0, NJB)
        lax.fori_loop(done, ready, jbody, 0)
        return ready

    lax.fori_loop(0, NS2, conv2_body, 0)
    for slot in range(2):
        for sub in range(NSUB):
            out_copy(slot, sub, 0, 0).wait()


@jax.jit
def pallas_standalone__seq2seq_rnn_t_joint__speech_kernel(x, w1, w2, g, w_f, w_g, w_o):
    anyspec = pl.BlockSpec(memory_space=pl.ANY)
    return pl.pallas_call(
        _kernel,
        out_shape=jax.ShapeDtypeStruct((B, T2, NU, D), BF16),
        in_specs=[anyspec] * 7,
        out_specs=anyspec,
        scratch_shapes=[
            pltpu.VMEM((2, X_ROWS, 128), BF16),
            pltpu.VMEM((12, 2, XSR, 128), U32),
            pltpu.VMEM((12, 2, H_ROWS, 128), U32),
            pltpu.VMEM((2, B * FSTRIDE + 32, 128), BF16),
            pltpu.VMEM((NUSLOT, 2, UROWS, 128), BF16),
            pltpu.VMEM((2, JB, NU, D), BF16),
            pltpu.VMEM((2, KT, D, 128), BF16),
            pltpu.VMEM((2, KT, D, 128), BF16),
            pltpu.VMEM((B, NU, D), BF16),
            pltpu.VMEM((D, D), BF16),
            pltpu.VMEM((D, D), BF16),
            pltpu.VMEM((D, D), BF16),
            pltpu.VMEM((B, NU, D), F32),
            pltpu.SemaphoreType.DMA((N_XSEM,)),
            pltpu.SemaphoreType.DMA((2 * NWP + 2,)),
            pltpu.SemaphoreType.DMA((4,)),
            pltpu.SemaphoreType.DMA((2 * NSUB,)),
        ],
        compiler_params=pltpu.CompilerParams(vmem_limit_bytes=110 * 1024 * 1024),
    )(x, w1, w2, g, w_f, w_g, w_o)
```

```python
import jax
import jax.numpy as jnp
from jax import lax
import jax.experimental.pallas as pl
import jax.experimental.pallas.tpu as pltpu

F32 = jnp.float32
BF16 = jnp.bfloat16
U32 = jnp.uint32

B, T, D, KT, NU = 2, 16000, 256, 31, 8
T1 = T // 2
T2 = T // 4
NB1 = 336
NB2 = 168
MC = 48
NS1 = B * NB1 // MC
NS2 = B * NB2 // MC
XB = 48
XSTRIDE = NB1 * 48
FSTRIDE = NB2 * 24
XSR = 2 * MC + 8
SRCV = 12 * XSR + 32
X_ROWS = -(-2 * (24 * MC * (NS1 - 1) + SRCV) // 64) * 64
HPAD = 8
H_ROWS = HPAD + B * NB1 + 8
UROWS = 512 + 16
NWP = 4
XWAIT = (0, 1, 3, 7)
JB = 12 * MC
NJB = FSTRIDE // JB
JSUB = (112, 112, 112, 112, 96, 32)
NSUB = len(JSUB)
JOFF = [sum(JSUB[:_i]) for _i in range(NSUB)]
assert sum(JSUB) == JB and JSUB[-1] == FSTRIDE - T2

BR_ORDER = (1, 2, 0, 3)
INNER = [(a2, a3, a4) for a2 in (1, 0, 2) for a3 in (1, 0, 2) for a4 in (1, 0, 2)]


def _is_raw(a1, a):
    return a1 in (0, 3) and all(v != 1 for v in a)


_USLOT = {}
for _a1 in range(4):
    for _a in INNER:
        if not _is_raw(_a1, _a):
            _USLOT[(_a1,) + _a] = len(_USLOT)
NUSLOT = len(_USLOT)


def _x_pieces():
    pieces, done = [], 0
    for i in range(len(XWAIT)):
        last = (XWAIT[i + 1] if i + 1 < len(XWAIT) else NS1) - 1
        need = 2 * (24 * MC * last + SRCV) - XB
        if last == NS1 - 1:
            need = B * XSTRIDE
        cur = []
        for b in range(B):
            lo = max(done - b * XSTRIDE, 0)
            hi = min(need - b * XSTRIDE, T)
            if hi > lo:
                cur.append((b, lo, hi))
        done = need
        pieces.append(cur)
    return pieces


X_PIECES = _x_pieces()
N_XSEM = 2 * sum(len(p) for p in X_PIECES)


def _sgn(t):
    return (-1) ** sum(1 for v in t if v == 2)


def _prod_of(sset, off):
    base = sum(d for d in (4, 2, 1) if d not in sset)
    rem = off - base
    return tuple((2 if rem & d else 0) if d in sset else 1 for d in (4, 2, 1))


def _gelu_scaled(v, k):
    c0 = 0.7978845608028654 * k
    c1 = 0.7978845608028654 * 0.044715 * k * k * k
    inner = v * (c0 + c1 * (v * v))
    hx = (0.5 * k) * v
    return hx + hx * jnp.tanh(inner)


def _kernel(x_hbm, w1_hbm, w2_hbm, g_hbm, wf_hbm, wg_hbm, wo_hbm, o_hbm,
            raw_ref, xs_ref, hs_ref, f_ref, u_ref, ob_ref, wr1_ref, wr2_ref,
            g_ref, wf_ref, wg_ref, wo_ref, ge_ref,
            xsem, wsem, ssem, osem):
    raw_u = raw_ref.bitcast(U32)
    f_u = f_ref.bitcast(U32)
    u_u = u_ref.bitcast(U32)
    wr1_u = wr1_ref.bitcast(U32)
    wr2_u = wr2_ref.bitcast(U32)

    def x_copies(k):
        out = []
        si = 2 * sum(len(p) for p in X_PIECES[:k])
        for (b, lo, hi) in X_PIECES[k]:
            for h in range(2):
                out.append(pltpu.make_async_copy(
                    x_hbm.at[b, pl.ds(lo, hi - lo), pl.ds(128 * h, 128)],
                    raw_ref.at[h, pl.ds(XB + b * XSTRIDE + lo, hi - lo), :],
                    xsem.at[si]))
                si += 1
        return out

    wrows = D // NWP

    def w1_copies(i):
        r0 = i * wrows
        if not isinstance(r0, int):
            r0 = pl.multiple_of(r0, wrows)
        return [pltpu.make_async_copy(
            w1_hbm.at[:, pl.ds(r0, wrows), pl.ds(128 * h, 128)],
            wr1_ref.at[h, :, pl.ds(r0, wrows), :], wsem.at[2 * i + h]) for h in range(2)]

    w2_copies = [pltpu.make_async_copy(
        w2_hbm.at[:, :, pl.ds(128 * h, 128)], wr2_ref.at[h], wsem.at[2 * NWP + h])
        for h in range(2)]

    small = [pltpu.make_async_copy(s, d, ssem.at[i]) for i, (s, d) in enumerate(
        [(g_hbm, g_ref), (wf_hbm, wf_ref), (wg_hbm, wg_ref), (wo_hbm, wo_ref)])]

    for i in range(2):
        for c in w1_copies(i):
            c.start()

    def zero_raw(lo, hi):
        for h in range(2):
            raw_u[h, pl.ds(lo // 2, (hi - lo) // 2), :] = jnp.zeros(((hi - lo) // 2, 128), U32)

    zero_raw(0, XB)
    zero_raw(XB + T, XB + XSTRIDE)
    zero_raw(XB + XSTRIDE + T, X_ROWS)
    hs_ref[:, :, pl.ds(0, HPAD), :] = jnp.zeros((12, 2, HPAD, 128), U32)
    hs_ref[:, :, pl.ds(HPAD + B * NB1, 8), :] = jnp.zeros((12, 2, 8, 128), U32)

    def w_unit(wr_u, rg, ph, h, branches):
        r0 = pl.multiple_of(rg * 8, 8)
        u0 = pl.multiple_of(ph * 256 + rg * 16, 16)

        def tap(j):
            if 2 * j - 1 + ph < 0:
                return jnp.zeros((16, 128), F32)
            tu = wr_u[h, 2 * j - 1 + ph, pl.ds(r0, 8), :]
            return pltpu.bitcast(tu, BF16).astype(F32)

        def rec(a1, d, ws, prefix):
            if d == 0:
                if not _is_raw(a1, prefix):
                    u_ref[_USLOT[(a1,) + prefix], h, pl.ds(u0, 16), :] = ws[0].astype(BF16)
                return
            lo, hi = ws[:d], ws[d:]
            rec(a1, d // 2, lo, prefix + (0,))
            rec(a1, d // 2, [a + b for a, b in zip(lo, hi)], prefix + (1,))
            rec(a1, d // 2, hi, prefix + (2,))

        lo = [tap(j) for j in range(8)]
        hi = [tap(j + 8) for j in range(8)]
        for a1 in branches:
            if a1 == 0:
                rec(0, 4, lo, ())
            elif a1 == 3:
                rec(3, 4, hi, ())
            elif a1 == 1:
                rec(1, 4, [a + b for a, b in zip(lo, hi)], ())
            else:
                rec(2, 4, [a - b for a, b in zip(lo, hi)], ())

    def w_rows(wr_u, rg_lo, rg_hi):
        for branches in ((1, 2), (0, 3)):
            def body(rg, carry, branches=branches):
                for ph in range(2):
                    for h in range(2):
                        w_unit(wr_u, rg, ph, h, branches)
                return carry
            lax.fori_loop(rg_lo, rg_hi, body, 0)

    def t_branch(st_ref, roff, branch):
        vals = {}

        def X(i):
            dl, r = divmod(2 * i - 16, 24)
            u = st_ref[r // 2, :, pl.ds(dl + roff, MC, stride=2), :]
            u = jnp.concatenate([u << 16, u & jnp.uint32(0xFFFF0000)], axis=0)
            return lax.bitcast_convert_type(u, F32)

        def Z(i):
            if branch == 0:
                return X(i) - X(i + 16)
            if branch == 1:
                return X(i + 8) + X(i + 16)
            if branch == 2:
                return X(i + 16) - X(i + 8)
            return X(i + 8) - X(i + 24)

        def put(sset, off, val):
            vals[_prod_of(sset, off)] = val

        z, a, b, d2 = {}, {}, {}, {}
        for n in range(15):
            z[n] = Z(n)
            if n == 7:
                put((), 7, z[7])
            if n - 1 in (6, 7):
                put((1,), n - 1, z[n - 1] - z[n])
            if 4 <= n - 2 <= 8:
                d2[n - 2] = z[n - 2] - z[n]
                if n - 2 in (5, 7):
                    put((2,), n - 2, d2[n - 2])
            if 4 <= n - 3 <= 7:
                put((2, 1), n - 3, d2[n - 3] - d2[n - 2])
            if n >= 4:
                a[n - 4] = z[n - 4] - z[n]
                if n - 4 in (3, 7):
                    put((4,), n - 4, a[n - 4])
            if n - 5 in (2, 3, 6, 7):
                put((4, 1), n - 5, a[n - 5] - a[n - 4])
            if n >= 6:
                b[n - 6] = a[n - 6] - a[n - 4]
                if n - 6 in (1, 3, 5, 7):
                    put((4, 2), n - 6, b[n - 6])
            if n >= 7:
                put((4, 2, 1), n - 7, b[n - 7] - b[n - 6])
        return vals

    def mm_branch(wr_u, branch, vals, qv, store_out):
        pv = {}
        for a in INNER:
            a2, a3, a4 = a
            s_in = _sgn(a)
            l0 = 0
            if _is_raw(branch, a):
                j = 8 * (branch // 3) + 4 * (a2 // 2) + 2 * (a3 // 2) + a4 // 2
                taps = [2 * j - 1, 2 * j]
                if j == 0:
                    taps, l0 = [0], 2
                rhs_u = jnp.concatenate(
                    [jnp.concatenate([wr_u[h, t] for t in taps], axis=0) for h in range(2)],
                    axis=1)
            else:
                rhs_u = jnp.concatenate(
                    [u_u[_USLOT[(branch,) + a], h, pl.ds(0, 256), :] for h in range(2)],
                    axis=1)
            lhs = jnp.concatenate(
                [vals[a][l] for l in range(l0, 4)], axis=1).astype(BF16)
            val = jnp.dot(lhs, pltpu.bitcast(rhs_u, BF16), preferred_element_type=F32)
            deps = []
            if a4 != 1:
                deps.append((a2, a3, 1))
                if a3 != 1:
                    deps.append((a2, 1, a4))
                    if a2 != 1:
                        deps.append((1, a3, a4))
            for dslot in deps:
                if _sgn(dslot) == s_in:
                    val = val + pv[dslot]
                else:
                    val = val - pv[dslot]
            if len(deps) < 3:
                pv[a] = val
                continue
            rp = (a2 // 2) * 4 + (a3 // 2) * 2 + (a4 // 2)
            if branch == 1:
                qv[rp] = val
                continue
            scl = 1.0
            if branch == 2:
                y, o, scl = qv[rp] - val, 1, 0.5
                qv[rp] = (qv[rp] + val) * 0.5
            elif branch == 0:
                y, o = qv[rp] + val, 0
            else:
                y, o = qv[rp] - val, 2
            gl = _gelu_scaled(y, scl * s_in)
            if a4 == 0:
                pv[a] = gl
                continue
            ev = pv[(a2, a3, 0)]
            lo = lax.bitcast_convert_type(ev.astype(BF16).astype(F32), U32) >> 16
            hi = lax.bitcast_convert_type(gl.astype(BF16).astype(F32), U32)
            pk = hi | lo
            for h in range(2):
                store_out(4 * o + rp // 2, h, pk[:, 128 * h:128 * (h + 1)])

    def conv_block(wr_u, st_ref, roff, store_out):
        qv = {}
        for br in BR_ORDER:
            mm_branch(wr_u, br, t_branch(st_ref, roff, br), qv, store_out)

    per = 16 // NWP

    def w1_piece(i, carry):
        for c in w1_copies(i):
            c.wait()

        @pl.when(i + 2 < NWP)
        def _():
            for c in w1_copies(i + 2):
                c.start()

        @pl.when(i == NWP - 2)
        def _():
            for c in x_copies(0):
                c.start()
        w_rows(wr1_u, i * per, (i + 1) * per)
        return carry

    lax.fori_loop(0, NWP, w1_piece, 0)

    def conv1_body(s, carry):
        for k, sk in enumerate(XWAIT):
            @pl.when(s == sk)
            def _():
                for c in x_copies(k):
                    c.wait()
                if k + 1 < len(X_PIECES):
                    for c in x_copies(k + 1):
                        c.start()
                else:
                    for c in w2_copies + small:
                        c.start()

        srcb = pl.multiple_of((24 * MC) * s, 32)
        src = raw_u.at[:, pl.ds(srcb, SRCV), :]
        for q in range(12):
            xs_ref[q] = src[:, pl.ds(12 + q, XSR, stride=12), :]

        hb = pl.multiple_of(HPAD + MC * s, 8)

        def store_h(qq, h, val):
            hs_ref[qq, h, pl.ds(hb, MC), :] = val

        conv_block(wr1_u, xs_ref, 1, store_h)
        return carry

    lax.fori_loop(0, NS1, conv1_body, 0)

    for c in w2_copies:
        c.wait()
    w_rows(wr2_u, 0, 16)

    nfull, rem = divmod(T1, 24)
    for b in range(B):
        r0 = HPAD + b * NB1 + nfull
        hs_ref[pl.ds(rem // 2, 12 - rem // 2), :, pl.ds(r0, 1), :] = jnp.zeros(
            (12 - rem // 2, 2, 1, 128), U32)
        hs_ref[:, :, pl.ds(r0 + 1, NB1 - nfull - 1), :] = jnp.zeros(
            (12, 2, NB1 - nfull - 1, 128), U32)

    for c in small:
        c.wait()
    for b in range(B):
        ge_ref[b] = jnp.dot(g_ref[b], wg_ref[...], preferred_element_type=F32)

    def out_copy(gi, sub):
        t0 = (gi % NJB) * JB + JOFF[sub]
        if sub == NSUB - 1:
            t0 = jnp.minimum(t0, T2 - JSUB[sub])
        slot = gi % 4
        return pltpu.make_async_copy(
            ob_ref.at[slot, pl.ds(JOFF[sub], JSUB[sub])],
            o_hbm.at[gi // NJB, pl.ds(t0, JSUB[sub])], osem.at[slot * NSUB + sub])

    def tile_dma(gi, sub, op):
        if sub < NSUB - 1:
            op(out_copy(gi, sub))
        else:
            @pl.when(gi % NJB != NJB - 1)
            def _():
                op(out_copy(gi, sub))

    def jtile(gi):
        ge = ge_ref[gi // NJB]
        r0 = pl.multiple_of(gi * (JB // 2), 32)
        fsrc = f_u.at[:, pl.ds(r0, JB // 2), :]
        f = jnp.concatenate(
            [pltpu.bitcast(fsrc[h], BF16) for h in range(2)], axis=1)
        fe = jnp.dot(f, wf_ref[...], preferred_element_type=F32)
        for sub in range(NSUB):
            js = JSUB[sub]
            fs = fe[JOFF[sub]:JOFF[sub] + js]
            jj = jnp.tanh(fs[:, None, :] + ge[None, :, :]).reshape(js * NU, D).astype(BF16)
            o = jnp.dot(jj, wo_ref[...], preferred_element_type=F32)
            ob_ref[gi % 4, pl.ds(JOFF[sub], js)] = o.reshape(js, NU, D).astype(BF16)
            tile_dma(gi, sub, lambda cp: cp.start())

    def conv2_body(c, carry):
        @pl.when(c >= 2)
        def _():
            for i in range(2):
                for sub in range(NSUB):
                    tile_dma(2 * (c - 2) + i, sub, lambda cp: cp.wait())

        hb = pl.multiple_of(2 * MC * c, 32)
        hsv = hs_ref.at[:, :, pl.ds(hb, 2 * MC + 16), :]
        fb = pl.multiple_of(12 * MC * c, 32)
        dst = f_u.at[:, pl.ds(fb, 12 * MC + 16), :]

        def store_f(qq, h, val):
            dst[h, pl.ds(qq, MC, stride=12), :] = val

        conv_block(wr2_u, hsv, HPAD, store_f)
        for i in range(2):
            jtile(2 * c + i)
        return carry

    lax.fori_loop(0, NS2, conv2_body, 0)
    for gi in range(2 * NS2 - 4, 2 * NS2):
        for sub in range(NSUB):
            if sub < NSUB - 1 or gi % NJB != NJB - 1:
                out_copy(gi, sub).wait()


@jax.jit
def pallas_standalone__seq2seq_rnn_t_joint__speech_kernel(x, w1, w2, g, w_f, w_g, w_o):
    anyspec = pl.BlockSpec(memory_space=pl.ANY)
    return pl.pallas_call(
        _kernel,
        out_shape=jax.ShapeDtypeStruct((B, T2, NU, D), BF16),
        in_specs=[anyspec] * 7,
        out_specs=anyspec,
        scratch_shapes=[
            pltpu.VMEM((2, X_ROWS, 128), BF16),
            pltpu.VMEM((12, 2, XSR, 128), U32),
            pltpu.VMEM((12, 2, H_ROWS, 128), U32),
            pltpu.VMEM((2, B * FSTRIDE + 32, 128), BF16),
            pltpu.VMEM((NUSLOT, 2, UROWS, 128), BF16),
            pltpu.VMEM((4, JB, NU, D), BF16),
            pltpu.VMEM((2, KT, D, 128), BF16),
            pltpu.VMEM((2, KT, D, 128), BF16),
            pltpu.VMEM((B, NU, D), BF16),
            pltpu.VMEM((D, D), BF16),
            pltpu.VMEM((D, D), BF16),
            pltpu.VMEM((D, D), BF16),
            pltpu.VMEM((B, NU, D), F32),
            pltpu.SemaphoreType.DMA((N_XSEM,)),
            pltpu.SemaphoreType.DMA((2 * NWP + 2,)),
            pltpu.SemaphoreType.DMA((4,)),
            pltpu.SemaphoreType.DMA((4 * NSUB,)),
        ],
        compiler_params=pltpu.CompilerParams(vmem_limit_bytes=110 * 1024 * 1024),
    )(x, w1, w2, g, w_f, w_g, w_o)
```

```python
import jax
import jax.numpy as jnp
from jax import lax
import jax.experimental.pallas as pl
import jax.experimental.pallas.tpu as pltpu

F32 = jnp.float32
BF16 = jnp.bfloat16
U32 = jnp.uint32

B, T, D, KT, NU = 2, 16000, 256, 31, 8
T1 = T // 2
T2 = T // 4
NB1 = 336
NB2 = 168
MC = 48
NS1 = B * NB1 // MC
NS2 = B * NB2 // MC
XB = 48
XSTRIDE = NB1 * 48
FSTRIDE = NB2 * 24
XSR = 2 * MC + 8
SRCV = 12 * XSR + 32
X_ROWS = -(-2 * (24 * MC * (NS1 - 1) + SRCV) // 64) * 64
HPAD = 8
H_ROWS = HPAD + B * NB1 + 8
UROWS = 512 + 16
NWP = 4
XWAIT = (0, 1, 3, 7)
JB = 12 * MC
NJB = FSTRIDE // JB
JSUB = (112, 112, 112, 112, 96, 32)
NSUB = len(JSUB)
JOFF = [sum(JSUB[:_i]) for _i in range(NSUB)]
assert sum(JSUB) == JB and JSUB[-1] == FSTRIDE - T2

BR_ORDER = (1, 2, 0, 3)
INNER = [(a2, a3, a4) for a2 in (1, 0, 2) for a3 in (1, 0, 2) for a4 in (1, 0, 2)]


def _is_raw(a1, a):
    return a1 in (0, 3) and all(v != 1 for v in a)


_USLOT = {}
for _a1 in range(4):
    for _a in INNER:
        if not _is_raw(_a1, _a):
            _USLOT[(_a1,) + _a] = len(_USLOT)
NUSLOT = len(_USLOT)


def _x_pieces():
    pieces, done = [], 0
    for i in range(len(XWAIT)):
        last = (XWAIT[i + 1] if i + 1 < len(XWAIT) else NS1) - 1
        need = 2 * (24 * MC * last + SRCV) - XB
        if last == NS1 - 1:
            need = B * XSTRIDE
        cur = []
        for b in range(B):
            lo = max(done - b * XSTRIDE, 0)
            hi = min(need - b * XSTRIDE, T)
            if hi > lo:
                cur.append((b, lo, hi))
        done = need
        pieces.append(cur)
    return pieces


X_PIECES = _x_pieces()
N_XSEM = 2 * sum(len(p) for p in X_PIECES)


def _sgn(t):
    return (-1) ** sum(1 for v in t if v == 2)


def _prod_of(sset, off):
    base = sum(d for d in (4, 2, 1) if d not in sset)
    rem = off - base
    return tuple((2 if rem & d else 0) if d in sset else 1 for d in (4, 2, 1))


def _gelu_scaled(v, k):
    c0 = 0.7978845608028654 * k
    c1 = 0.7978845608028654 * 0.044715 * k * k * k
    inner = v * (c0 + c1 * (v * v))
    hx = (0.5 * k) * v
    return hx + hx * jnp.tanh(inner)


def _kernel(x_hbm, w1_hbm, w2_hbm, g_hbm, wf_hbm, wg_hbm, wo_hbm, o_hbm,
            raw_ref, xs_ref, hs_ref, f_ref, u_ref, ob_ref, wr1_ref, wr2_ref,
            g_ref, wf_ref, wg_ref, wo_ref, ge_ref,
            xsem, wsem, ssem, osem):
    raw_u = raw_ref.bitcast(U32)
    f_u = f_ref.bitcast(U32)
    u_u = u_ref.bitcast(U32)
    wr1_u = wr1_ref.bitcast(U32)
    wr2_u = wr2_ref.bitcast(U32)

    def x_copies(k):
        out = []
        si = 2 * sum(len(p) for p in X_PIECES[:k])
        for (b, lo, hi) in X_PIECES[k]:
            for h in range(2):
                out.append(pltpu.make_async_copy(
                    x_hbm.at[b, pl.ds(lo, hi - lo), pl.ds(128 * h, 128)],
                    raw_ref.at[h, pl.ds(XB + b * XSTRIDE + lo, hi - lo), :],
                    xsem.at[si]))
                si += 1
        return out

    wrows = D // NWP

    def w1_copies(i):
        r0 = i * wrows
        if not isinstance(r0, int):
            r0 = pl.multiple_of(r0, wrows)
        return [pltpu.make_async_copy(
            w1_hbm.at[:, pl.ds(r0, wrows), pl.ds(128 * h, 128)],
            wr1_ref.at[h, :, pl.ds(r0, wrows), :], wsem.at[2 * i + h]) for h in range(2)]

    w2_copies = [pltpu.make_async_copy(
        w2_hbm.at[:, :, pl.ds(128 * h, 128)], wr2_ref.at[h], wsem.at[2 * NWP + h])
        for h in range(2)]

    small = [pltpu.make_async_copy(s, d, ssem.at[i]) for i, (s, d) in enumerate(
        [(g_hbm, g_ref), (wf_hbm, wf_ref), (wg_hbm, wg_ref), (wo_hbm, wo_ref)])]

    for i in range(2):
        for c in w1_copies(i):
            c.start()

    def zero_raw(lo, hi):
        for h in range(2):
            raw_u[h, pl.ds(lo // 2, (hi - lo) // 2), :] = jnp.zeros(((hi - lo) // 2, 128), U32)

    zero_raw(0, XB)
    zero_raw(XB + T, XB + XSTRIDE)
    zero_raw(XB + XSTRIDE + T, X_ROWS)
    hs_ref[:, :, pl.ds(0, HPAD), :] = jnp.zeros((12, 2, HPAD, 128), U32)
    hs_ref[:, :, pl.ds(HPAD + B * NB1, 8), :] = jnp.zeros((12, 2, 8, 128), U32)

    def w_unit(wr_u, rg, ph, h, branches):
        r0 = pl.multiple_of(rg * 8, 8)
        u0 = pl.multiple_of(ph * 256 + rg * 16, 16)

        def tap(j):
            if 2 * j - 1 + ph < 0:
                return jnp.zeros((16, 128), F32)
            tu = wr_u[h, 2 * j - 1 + ph, pl.ds(r0, 8), :]
            return pltpu.bitcast(tu, BF16).astype(F32)

        def rec(a1, d, ws, prefix):
            if d == 0:
                if not _is_raw(a1, prefix):
                    u_ref[_USLOT[(a1,) + prefix], h, pl.ds(u0, 16), :] = ws[0].astype(BF16)
                return
            lo, hi = ws[:d], ws[d:]
            rec(a1, d // 2, lo, prefix + (0,))
            rec(a1, d // 2, [a + b for a, b in zip(lo, hi)], prefix + (1,))
            rec(a1, d // 2, hi, prefix + (2,))

        lo = [tap(j) for j in range(8)]
        hi = [tap(j + 8) for j in range(8)]
        for a1 in branches:
            if a1 == 0:
                rec(0, 4, lo, ())
            elif a1 == 3:
                rec(3, 4, hi, ())
            elif a1 == 1:
                rec(1, 4, [a + b for a, b in zip(lo, hi)], ())
            else:
                rec(2, 4, [a - b for a, b in zip(lo, hi)], ())

    def w_rows(wr_u, rg_lo, rg_hi):
        for branches in ((1, 2), (0, 3)):
            def body(rg, carry, branches=branches):
                for ph in range(2):
                    for h in range(2):
                        w_unit(wr_u, rg, ph, h, branches)
                return carry
            lax.fori_loop(rg_lo, rg_hi, body, 0)

    def t_branch(st_ref, roff, branch):
        vals = {}

        def X(i):
            dl, r = divmod(2 * i - 16, 24)
            u = st_ref[r // 2, :, pl.ds(dl + roff, MC, stride=2), :]
            u = jnp.concatenate([u << 16, u & jnp.uint32(0xFFFF0000)], axis=0)
            return lax.bitcast_convert_type(u, F32)

        def Z(i):
            if branch == 0:
                return X(i) - X(i + 16)
            if branch == 1:
                return X(i + 8) + X(i + 16)
            if branch == 2:
                return X(i + 16) - X(i + 8)
            return X(i + 8) - X(i + 24)

        def put(sset, off, val):
            vals[_prod_of(sset, off)] = val

        z, a, b, d2 = {}, {}, {}, {}
        for n in range(15):
            z[n] = Z(n)
            if n == 7:
                put((), 7, z[7])
            if n - 1 in (6, 7):
                put((1,), n - 1, z[n - 1] - z[n])
            if 4 <= n - 2 <= 8:
                d2[n - 2] = z[n - 2] - z[n]
                if n - 2 in (5, 7):
                    put((2,), n - 2, d2[n - 2])
            if 4 <= n - 3 <= 7:
                put((2, 1), n - 3, d2[n - 3] - d2[n - 2])
            if n >= 4:
                a[n - 4] = z[n - 4] - z[n]
                if n - 4 in (3, 7):
                    put((4,), n - 4, a[n - 4])
            if n - 5 in (2, 3, 6, 7):
                put((4, 1), n - 5, a[n - 5] - a[n - 4])
            if n >= 6:
                b[n - 6] = a[n - 6] - a[n - 4]
                if n - 6 in (1, 3, 5, 7):
                    put((4, 2), n - 6, b[n - 6])
            if n >= 7:
                put((4, 2, 1), n - 7, b[n - 7] - b[n - 6])
        return vals

    def mm_branch(wr_u, branch, vals, qv, store_out):
        pv = {}
        for a in INNER:
            a2, a3, a4 = a
            s_in = _sgn(a)
            l0 = 0
            if _is_raw(branch, a):
                j = 8 * (branch // 3) + 4 * (a2 // 2) + 2 * (a3 // 2) + a4 // 2
                taps = [2 * j - 1, 2 * j]
                if j == 0:
                    taps, l0 = [0], 2
                rhs_u = jnp.concatenate(
                    [jnp.concatenate([wr_u[h, t] for t in taps], axis=0) for h in range(2)],
                    axis=1)
            else:
                rhs_u = jnp.concatenate(
                    [u_u[_USLOT[(branch,) + a], h, pl.ds(0, 256), :] for h in range(2)],
                    axis=1)
            lhs = jnp.concatenate(
                [vals[a][l] for l in range(l0, 4)], axis=1).astype(BF16)
            val = jnp.dot(lhs, pltpu.bitcast(rhs_u, BF16), preferred_element_type=F32)
            deps = []
            if a4 != 1:
                deps.append((a2, a3, 1))
                if a3 != 1:
                    deps.append((a2, 1, a4))
                    if a2 != 1:
                        deps.append((1, a3, a4))
            for dslot in deps:
                if _sgn(dslot) == s_in:
                    val = val + pv[dslot]
                else:
                    val = val - pv[dslot]
            if len(deps) < 3:
                pv[a] = val
                continue
            rp = (a2 // 2) * 4 + (a3 // 2) * 2 + (a4 // 2)
            if branch == 1:
                qv[rp] = val
                continue
            scl = 1.0
            if branch == 2:
                y, o, scl = qv[rp] - val, 1, 0.5
                qv[rp] = (qv[rp] + val) * 0.5
            elif branch == 0:
                y, o = qv[rp] + val, 0
            else:
                y, o = qv[rp] - val, 2
            gl = _gelu_scaled(y, scl * s_in)
            if a4 == 0:
                pv[a] = gl
                continue
            ev = pv[(a2, a3, 0)]
            lo = lax.bitcast_convert_type(ev.astype(BF16).astype(F32), U32) >> 16
            hi = lax.bitcast_convert_type(gl.astype(BF16).astype(F32), U32)
            pk = hi | lo
            for h in range(2):
                store_out(4 * o + rp // 2, h, pk[:, 128 * h:128 * (h + 1)])

    def conv_block(wr_u, st_ref, roff, store_out):
        qv = {}
        for br in BR_ORDER:
            mm_branch(wr_u, br, t_branch(st_ref, roff, br), qv, store_out)

    per = 16 // NWP

    def w1_piece(i, carry):
        for c in w1_copies(i):
            c.wait()

        @pl.when(i + 2 < NWP)
        def _():
            for c in w1_copies(i + 2):
                c.start()

        @pl.when(i == NWP - 2)
        def _():
            for c in x_copies(0):
                c.start()
        w_rows(wr1_u, i * per, (i + 1) * per)
        return carry

    lax.fori_loop(0, NWP, w1_piece, 0)

    def conv1_body(s, carry):
        srcb = pl.multiple_of((24 * MC) * s, 32)
        src = raw_u.at[:, pl.ds(srcb, SRCV), :]
        for q in range(12):
            xs_ref[q] = src[:, pl.ds(12 + q, XSR, stride=12), :]

        hb = pl.multiple_of(HPAD + MC * s, 8)

        def store_h(qq, h, val):
            hs_ref[qq, h, pl.ds(hb, MC), :] = val

        conv_block(wr1_u, xs_ref, 1, store_h)
        return carry

    def x_piece(k, lo):
        hi = NS1
        for kk in range(len(XWAIT)):
            @pl.when(k == kk)
            def _():
                for c in x_copies(kk):
                    c.wait()
                if kk + 1 < len(X_PIECES):
                    for c in x_copies(kk + 1):
                        c.start()
                else:
                    for c in w2_copies + small:
                        c.start()
            if kk + 1 < len(XWAIT):
                hi = jnp.where(k == kk, XWAIT[kk + 1], hi)
        lax.fori_loop(lo, hi, conv1_body, 0)
        return hi

    lax.fori_loop(0, len(XWAIT), x_piece, 0)

    for c in w2_copies:
        c.wait()
    w_rows(wr2_u, 0, 16)

    nfull, rem = divmod(T1, 24)
    for b in range(B):
        r0 = HPAD + b * NB1 + nfull
        hs_ref[pl.ds(rem // 2, 12 - rem // 2), :, pl.ds(r0, 1), :] = jnp.zeros(
            (12 - rem // 2, 2, 1, 128), U32)
        hs_ref[:, :, pl.ds(r0 + 1, NB1 - nfull - 1), :] = jnp.zeros(
            (12, 2, NB1 - nfull - 1, 128), U32)

    for c in small:
        c.wait()
    for b in range(B):
        ge_ref[b] = jnp.dot(g_ref[b], wg_ref[...], preferred_element_type=F32)

    def out_copy(gi, sub):
        t0 = (gi % NJB) * JB + JOFF[sub]
        if sub == NSUB - 1:
            t0 = jnp.minimum(t0, T2 - JSUB[sub])
        slot = gi % 4
        return pltpu.make_async_copy(
            ob_ref.at[slot, pl.ds(JOFF[sub], JSUB[sub])],
            o_hbm.at[gi // NJB, pl.ds(t0, JSUB[sub])], osem.at[slot * NSUB + sub])

    def tile_dma(gi, sub, op):
        if sub < NSUB - 1:
            op(out_copy(gi, sub))
        else:
            @pl.when(gi % NJB != NJB - 1)
            def _():
                op(out_copy(gi, sub))

    def jtile(gi):
        ge = ge_ref[gi // NJB]
        r0 = pl.multiple_of(gi * (JB // 2), 32)
        fsrc = f_u.at[:, pl.ds(r0, JB // 2), :]
        f = jnp.concatenate(
            [pltpu.bitcast(fsrc[h], BF16) for h in range(2)], axis=1)
        fe = jnp.dot(f, wf_ref[...], preferred_element_type=F32)
        for sub in range(NSUB):
            js = JSUB[sub]
            fs = fe[JOFF[sub]:JOFF[sub] + js]
            jj = jnp.tanh(fs[:, None, :] + ge[None, :, :]).reshape(js * NU, D).astype(BF16)
            o = jnp.dot(jj, wo_ref[...], preferred_element_type=F32)
            ob_ref[gi % 4, pl.ds(JOFF[sub], js)] = o.reshape(js, NU, D).astype(BF16)
            tile_dma(gi, sub, lambda cp: cp.start())

    def conv2_body(c, carry):
        @pl.when(c >= 2)
        def _():
            for i in range(2):
                for sub in range(NSUB):
                    tile_dma(2 * (c - 2) + i, sub, lambda cp: cp.wait())

        hb = pl.multiple_of(2 * MC * c, 32)
        hsv = hs_ref.at[:, :, pl.ds(hb, 2 * MC + 16), :]
        fb = pl.multiple_of(12 * MC * c, 32)
        dst = f_u.at[:, pl.ds(fb, 12 * MC + 16), :]

        def store_f(qq, h, val):
            dst[h, pl.ds(qq, MC, stride=12), :] = val

        conv_block(wr2_u, hsv, HPAD, store_f)
        for i in range(2):
            jtile(2 * c + i)
        return carry

    lax.fori_loop(0, NS2, conv2_body, 0)
    for gi in range(2 * NS2 - 4, 2 * NS2):
        for sub in range(NSUB):
            if sub < NSUB - 1 or gi % NJB != NJB - 1:
                out_copy(gi, sub).wait()


@jax.jit
def pallas_standalone__seq2seq_rnn_t_joint__speech_kernel(x, w1, w2, g, w_f, w_g, w_o):
    anyspec = pl.BlockSpec(memory_space=pl.ANY)
    return pl.pallas_call(
        _kernel,
        out_shape=jax.ShapeDtypeStruct((B, T2, NU, D), BF16),
        in_specs=[anyspec] * 7,
        out_specs=anyspec,
        scratch_shapes=[
            pltpu.VMEM((2, X_ROWS, 128), BF16),
            pltpu.VMEM((12, 2, XSR, 128), U32),
            pltpu.VMEM((12, 2, H_ROWS, 128), U32),
            pltpu.VMEM((2, B * FSTRIDE + 32, 128), BF16),
            pltpu.VMEM((NUSLOT, 2, UROWS, 128), BF16),
            pltpu.VMEM((4, JB, NU, D), BF16),
            pltpu.VMEM((2, KT, D, 128), BF16),
            pltpu.VMEM((2, KT, D, 128), BF16),
            pltpu.VMEM((B, NU, D), BF16),
            pltpu.VMEM((D, D), BF16),
            pltpu.VMEM((D, D), BF16),
            pltpu.VMEM((D, D), BF16),
            pltpu.VMEM((B, NU, D), F32),
            pltpu.SemaphoreType.DMA((N_XSEM,)),
            pltpu.SemaphoreType.DMA((2 * NWP + 2,)),
            pltpu.SemaphoreType.DMA((4,)),
            pltpu.SemaphoreType.DMA((4 * NSUB,)),
        ],
        compiler_params=pltpu.CompilerParams(vmem_limit_bytes=110 * 1024 * 1024),
    )(x, w1, w2, g, w_f, w_g, w_o)
```
